```python
import os as _os
_os.environ.setdefault("JAX_PLATFORMS", "cpu")
import jax
import jax.numpy as jnp

def _softmax(x, axis=-1):
    return jax.nn.softmax(x, axis=axis)
def _gelu(x):
    return jax.nn.gelu(x, approximate=True)
def _silu(x):
    return jax.nn.silu(x)
def _sigmoid(x):
    return jax.nn.sigmoid(x)
def _layernorm(x, axis=-1, eps=1e-5):
    m = jnp.mean(x, axis=axis, keepdims=True)
    v = jnp.var(x, axis=axis, keepdims=True)
    return (x - m) / jnp.sqrt(v + eps)
def _scatter_add(tgt, idx, src, axis=0):
    return tgt.at[idx].add(src)
def _segment_sum(src, seg, n):
    return jax.ops.segment_sum(src, seg, n)
class _Rng:
    def __init__(self, key):
        self._k = key
    def _next(self):
        self._k, sub = jax.random.split(self._k)
        return sub
    def normal(self, shape):
        return jax.random.normal(self._next(), shape, dtype=jnp.bfloat16)
    def randint(self, lo, hi, shape):
        return jax.random.randint(self._next(), shape, lo, hi, dtype=jnp.int32)
    def uniform(self, shape, lo=0.0, hi=1.0):
        return jax.random.uniform(self._next(), shape, jnp.bfloat16, lo, hi)
    def permutation(self, n):
        return jax.random.permutation(self._next(), n)


kernel_name = 'standalone__mha_softmax__near_ridge'

def setup_inputs():
    _rng = _Rng(jax.random.key(int.from_bytes(__import__("os").urandom(4), "little")))
    _w = (lambda a: (lambda t: t.astype(jnp.bfloat16) if jnp.issubdtype(t.dtype, jnp.floating) else t)(jnp.asarray(a)))
    B, H, Sq, Sk, D = 8, 16, 192, 1024, 256
    return {
        "q": _w((lambda *s: _rng.normal(s) * 0.4)(B, H, Sq, D)),
        "k": _w((lambda *s: _rng.normal(s) * 0.4)(B, H, Sk, D)),
        "v": _w((lambda *s: _rng.normal(s) * 0.05)(B, H, Sk, D)),
    }

def reference(q, k, v):
    scale = q.shape[-1] ** -0.5
    scores = jnp.einsum("bhqd,bhkd->bhqk", q, k) * scale
    p = _softmax(scores, axis=-1)
    return jnp.einsum("bhqk,bhkd->bhqd", p, v)
```

```python
import functools

import jax
import jax.numpy as jnp
import jax.experimental.pallas as pl
import jax.experimental.pallas.tpu as pltpu


def _head(q, k, v, scale):
    s = jax.lax.dot_general(
        q, k, (((1,), (1,)), ((), ())), preferred_element_type=jnp.float32
    )
    s = s * scale
    m = jnp.max(s, axis=-1, keepdims=True)
    p = jnp.exp(s - m)
    l = jnp.sum(p, axis=-1, keepdims=True)
    o = jnp.dot(p.astype(v.dtype), v, preferred_element_type=jnp.float32)
    return o / l


def _kernel(q_hbm, k_hbm, v_hbm, o_hbm, qbuf, kbuf, vbuf, obuf, qsem, ksem, vsem, osem,
            *, hb, nbuf, scale):
    n = k_hbm.shape[0] // hb

    def in_copies(i, slot):
        sl = pl.ds(i * hb, hb)
        return (
            pltpu.make_async_copy(q_hbm.at[sl], qbuf.at[slot], qsem.at[slot]),
            pltpu.make_async_copy(k_hbm.at[sl], kbuf.at[slot], ksem.at[slot]),
            pltpu.make_async_copy(v_hbm.at[sl], vbuf.at[slot], vsem.at[slot]),
        )

    def out_copy(lo, hi, j):
        sl = pl.ds(lo * hb, (hi - lo) * hb)
        return pltpu.make_async_copy(obuf.at[sl], o_hbm.at[sl], osem.at[j])

    def compute(i, slot):
        for h in range(hb):
            o = _head(qbuf[slot, h], kbuf[slot, h], vbuf[slot, h], scale)
            obuf[i * hb + h] = o.astype(obuf.dtype)

    for j in range(nbuf - 1):
        for c in in_copies(j, j):
            c.start()

    def body(i, carry):
        nxt = i + nbuf - 1

        @pl.when(nxt < n)
        def _():
            for c in in_copies(nxt, nxt % nbuf):
                c.start()

        slot = i % nbuf
        for c in in_copies(i, slot):
            c.wait()
        compute(i, slot)
        return carry

    jax.lax.fori_loop(0, n - 1, body, 0)

    w0 = out_copy(0, n - 1, 0)
    w0.start()
    last_slot = (n - 1) % nbuf
    for c in in_copies(n - 1, last_slot):
        c.wait()
    compute(n - 1, last_slot)
    w1 = out_copy(n - 1, n, 1)
    w1.start()
    w0.wait()
    w1.wait()


@jax.jit
def pallas_standalone__mha_softmax__near_ridge_kernel(
    q: jax.Array,
    k: jax.Array,
    v: jax.Array,
):
    B, H, Sq, D = q.shape
    Sk = k.shape[2]
    BH = B * H
    hb = 2
    nbuf = 3
    assert BH % hb == 0 and BH // hb >= nbuf
    q3 = q.reshape(BH, Sq, D)
    k3 = k.reshape(BH, Sk, D)
    v3 = v.reshape(BH, Sk, D)
    scale = D ** -0.5

    out = pl.pallas_call(
        functools.partial(_kernel, hb=hb, nbuf=nbuf, scale=scale),
        in_specs=[pl.BlockSpec(memory_space=pl.ANY)] * 3,
        out_specs=pl.BlockSpec(memory_space=pl.ANY),
        out_shape=jax.ShapeDtypeStruct((BH, Sq, D), q.dtype),
        scratch_shapes=[
            pltpu.VMEM((nbuf, hb, Sq, D), q.dtype),
            pltpu.VMEM((nbuf, hb, Sk, D), k.dtype),
            pltpu.VMEM((nbuf, hb, Sk, D), v.dtype),
            pltpu.VMEM((BH, Sq, D), q.dtype),
            pltpu.SemaphoreType.DMA((nbuf,)),
            pltpu.SemaphoreType.DMA((nbuf,)),
            pltpu.SemaphoreType.DMA((nbuf,)),
            pltpu.SemaphoreType.DMA((2,)),
        ],
        compiler_params=pltpu.CompilerParams(vmem_limit_bytes=64 * 1024 * 1024),
    )(q3, k3, v3)
    return out.reshape(B, H, Sq, D)
```

```python
import functools

import jax
import jax.numpy as jnp
import jax.experimental.pallas as pl
import jax.experimental.pallas.tpu as pltpu


def _head(q, k, v, scale):
    s = jax.lax.dot_general(
        q, k, (((1,), (1,)), ((), ())), preferred_element_type=jnp.float32
    )
    s = s.astype(q.dtype).astype(jnp.float32) * scale
    m = jnp.max(s, axis=-1, keepdims=True)
    p = jnp.exp(s - m)
    l = jnp.sum(p, axis=-1, keepdims=True)
    o = jnp.dot(p.astype(v.dtype), v, preferred_element_type=jnp.float32)
    return o / l


def _kernel(q_hbm, k_hbm, v_hbm, o_hbm, qbuf, kbuf, vbuf, obuf, isem, osem, *, scale):
    nbuf, hb, sq, _ = qbuf.shape
    n = k_hbm.shape[0] // hb
    _, ncol, rows, _ = obuf.shape
    pieces = sq // rows

    def in_copies(i, slot):
        sl = pl.ds(i * hb, hb)
        return (
            pltpu.make_async_copy(q_hbm.at[sl], qbuf.at[slot], isem.at[slot]),
            pltpu.make_async_copy(k_hbm.at[sl], kbuf.at[slot], isem.at[slot]),
            pltpu.make_async_copy(v_hbm.at[sl], vbuf.at[slot], isem.at[slot]),
        )

    def out_copy(j):
        return pltpu.make_async_copy(obuf.at[:, j], o_hbm.at[:, j], osem.at[0])

    def compute(i, slot):
        for h in range(hb):
            o = _head(qbuf[slot, h], kbuf[slot, h], vbuf[slot, h], scale)
            o = o.astype(obuf.dtype)
            for t in range(pieces):
                c = (i * hb + h) * pieces + t
                obuf[c // ncol, c % ncol] = o[t * rows:(t + 1) * rows]

    for j in range(nbuf - 1):
        for cp in in_copies(j, j):
            cp.start()

    def body(i, carry):
        nxt = i + nbuf - 1

        @pl.when(nxt < n)
        def _():
            for cp in in_copies(nxt, nxt % nbuf):
                cp.start()

        slot = i % nbuf
        for cp in in_copies(i, slot):
            cp.wait()
        compute(i, slot)
        return carry

    jax.lax.fori_loop(0, n - 1, body, 0)

    late = hb * pieces
    for j in range(ncol - late):
        out_copy(j).start()
    last_slot = (n - 1) % nbuf
    for cp in in_copies(n - 1, last_slot):
        cp.wait()
    compute(n - 1, last_slot)
    for j in range(ncol - late, ncol):
        out_copy(j).start()
    for j in range(ncol):
        out_copy(j).wait()


@jax.jit
def pallas_standalone__mha_softmax__near_ridge_kernel(
    q: jax.Array,
    k: jax.Array,
    v: jax.Array,
):
    B, H, Sq, D = q.shape
    Sk = k.shape[2]
    BH = B * H
    hb = 2
    nbuf = 3
    rows = 32
    ncol = 64
    assert BH % hb == 0 and BH // hb >= nbuf
    assert Sq % rows == 0 and (BH * Sq) % (rows * ncol) == 0
    assert hb * (Sq // rows) <= ncol
    nrow = BH * Sq // (rows * ncol)

    out = pl.pallas_call(
        functools.partial(_kernel, scale=D ** -0.5),
        in_specs=[pl.BlockSpec(memory_space=pl.ANY)] * 3,
        out_specs=pl.BlockSpec(memory_space=pl.ANY),
        out_shape=jax.ShapeDtypeStruct((nrow, ncol, rows, D), q.dtype),
        scratch_shapes=[
            pltpu.VMEM((nbuf, hb, Sq, D), q.dtype),
            pltpu.VMEM((nbuf, hb, Sk, D), k.dtype),
            pltpu.VMEM((nbuf, hb, Sk, D), v.dtype),
            pltpu.VMEM((nrow, ncol, rows, D), q.dtype),
            pltpu.SemaphoreType.DMA((nbuf,)),
            pltpu.SemaphoreType.DMA((1,)),
        ],
        compiler_params=pltpu.CompilerParams(vmem_limit_bytes=64 * 1024 * 1024),
    )(q.reshape(BH, Sq, D), k.reshape(BH, Sk, D), v.reshape(BH, Sk, D))
    return out.reshape(B, H, Sq, D)
```
